```python
import os as _os
_os.environ.setdefault("JAX_PLATFORMS", "cpu")
import jax
import jax.numpy as jnp

def _softmax(x, axis=-1):
    return jax.nn.softmax(x, axis=axis)
def _gelu(x):
    return jax.nn.gelu(x, approximate=True)
def _silu(x):
    return jax.nn.silu(x)
def _sigmoid(x):
    return jax.nn.sigmoid(x)
def _layernorm(x, axis=-1, eps=1e-5):
    m = jnp.mean(x, axis=axis, keepdims=True)
    v = jnp.var(x, axis=axis, keepdims=True)
    return (x - m) / jnp.sqrt(v + eps)
def _scatter_add(tgt, idx, src, axis=0):
    return tgt.at[idx].add(src)
def _segment_sum(src, seg, n):
    return jax.ops.segment_sum(src, seg, n)
class _Rng:
    def __init__(self, key):
        self._k = key
    def _next(self):
        self._k, sub = jax.random.split(self._k)
        return sub
    def normal(self, shape):
        return jax.random.normal(self._next(), shape, dtype=jnp.bfloat16)
    def randint(self, lo, hi, shape):
        return jax.random.randint(self._next(), shape, lo, hi, dtype=jnp.int32)
    def uniform(self, shape, lo=0.0, hi=1.0):
        return jax.random.uniform(self._next(), shape, jnp.bfloat16, lo, hi)
    def permutation(self, n):
        return jax.random.permutation(self._next(), n)


kernel_name = 'gated_mix__ssm_conv_h3__ssm_conv_h3__prompt'

def setup_inputs():
    _rng = _Rng(jax.random.key(int.from_bytes(__import__("os").urandom(4), "little")))
    _w = (lambda a: (lambda t: t.astype(jnp.bfloat16) if jnp.issubdtype(t.dtype, jnp.floating) else t)(jnp.asarray(a)))
    def _A_setup():
        B, S, D = 1, 2048, 640
        ks = 4
        return {
            "q": _w((lambda *s: _rng.normal(s) * 0.05)(B, S, D)),
            "k": _w((lambda *s: _rng.normal(s) * 0.05)(B, S, D)),
            "v": _w((lambda *s: _rng.normal(s) * 0.05)(B, S, D)),
            "shift_k": _w((lambda *s: _rng.normal(s) * 0.05)(D, ks) * 0.5),
            "ssm_k": _w((lambda *s: _rng.normal(s) * 0.05)(D, S) * (1.0 / S ** 0.5)),
            "ssm_D": _w((lambda *s: _rng.normal(s) * 0.05)(D)),
        }
    _A_in = _A_setup()

    def _B_setup():
        B, S, D = 1, 2048, 640
        ks = 4
        return {
            "q": _w((lambda *s: _rng.normal(s) * 0.05)(B, S, D)),
            "k": _w((lambda *s: _rng.normal(s) * 0.05)(B, S, D)),
            "v": _w((lambda *s: _rng.normal(s) * 0.05)(B, S, D)),
            "shift_k": _w((lambda *s: _rng.normal(s) * 0.05)(D, ks) * 0.5),
            "ssm_k": _w((lambda *s: _rng.normal(s) * 0.05)(D, S) * (1.0 / S ** 0.5)),
            "ssm_D": _w((lambda *s: _rng.normal(s) * 0.05)(D)),
        }
    _B_in = _B_setup()

    return {
        "A_q": _A_in["q"],
        "A_k": _A_in["k"],
        "A_v": _A_in["v"],
        "A_shift_k": _A_in["shift_k"],
        "A_ssm_k": _A_in["ssm_k"],
        "A_ssm_D": _A_in["ssm_D"],
        "B_q": _B_in["q"],
        "B_k": _B_in["k"],
        "B_v": _B_in["v"],
        "B_shift_k": _B_in["shift_k"],
        "B_ssm_k": _B_in["ssm_k"],
        "B_ssm_D": _B_in["ssm_D"],
        "gate_w": _w((lambda *s: _rng.normal(s) * 0.05)(640) * 16.0),
    }

def reference(A_q, A_k, A_v, A_shift_k, A_ssm_k, A_ssm_D, B_q, B_k, B_v, B_shift_k, B_ssm_k, B_ssm_D, gate_w):
    def _A_ref(q, k, v, shift_k, ssm_k, ssm_D):
        B, S, D = q.shape
        ks = shift_k.shape[-1]
        k_pad = jnp.pad(k, ((0, 0), (ks - 1, 0), (0, 0)))
        k_shift = jnp.zeros_like(k)
        for t in range(ks):
            k_shift = k_shift + k_pad[:, t:t + S, :] * shift_k[:, ks - 1 - t][None, None, :]
        kv = k_shift * v
        L = 2 * S
        kv_pad = jnp.pad(kv, ((0, 0), (0, S), (0, 0)))
        kf_pad = jnp.pad(ssm_k, ((0, 0), (0, S)))
        kv_f = (lambda x, axes=(-2,-1): jnp.fft.rfft2(x.astype(jnp.float32), axes=axes))(kv_pad[:, None, :, :], axes=(1, 2))
        kf_f = (lambda x, axes=(-2,-1): jnp.fft.rfft2(x.astype(jnp.float32), axes=axes))(kf_pad[:, None, :], axes=(1, 2))
        kf_f = (lambda x, *d: x.transpose(*d))(kf_f, 1, 2, 0)
        y_f = kv_f * kf_f[None, :, :, :]
        y = (lambda x, s, axes=(-2,-1): jnp.fft.irfft2(x, s=s, axes=axes).astype(jnp.bfloat16))(y_f, (1, L), axes=(1, 2))[:, 0, :S, :]
        y = y + kv * ssm_D[None, None, :]
        return q * y

    def _B_ref(q, k, v, shift_k, ssm_k, ssm_D):
        B, S, D = q.shape
        ks = shift_k.shape[-1]
        k_pad = jnp.pad(k, ((0, 0), (ks - 1, 0), (0, 0)))
        k_shift = jnp.zeros_like(k)
        for t in range(ks):
            k_shift = k_shift + k_pad[:, t:t + S, :] * shift_k[:, ks - 1 - t][None, None, :]
        kv = k_shift * v
        L = 2 * S
        kv_pad = jnp.pad(kv, ((0, 0), (0, S), (0, 0)))
        kf_pad = jnp.pad(ssm_k, ((0, 0), (0, S)))
        kv_f = (lambda x, axes=(-2,-1): jnp.fft.rfft2(x.astype(jnp.float32), axes=axes))(kv_pad[:, None, :, :], axes=(1, 2))
        kf_f = (lambda x, axes=(-2,-1): jnp.fft.rfft2(x.astype(jnp.float32), axes=axes))(kf_pad[:, None, :], axes=(1, 2))
        kf_f = (lambda x, *d: x.transpose(*d))(kf_f, 1, 2, 0)
        y_f = kv_f * kf_f[None, :, :, :]
        y = (lambda x, s, axes=(-2,-1): jnp.fft.irfft2(x, s=s, axes=axes).astype(jnp.bfloat16))(y_f, (1, L), axes=(1, 2))[:, 0, :S, :]
        y = y + kv * ssm_D[None, None, :]
        return q * y

    x = A_q
    g = _sigmoid((x * gate_w).sum(-1, keepdims=True))
    a = _A_ref(x, A_k, A_v, A_shift_k, A_ssm_k, A_ssm_D)
    b = _B_ref(x, B_k, B_v, B_shift_k, B_ssm_k, B_ssm_D)
    return g * a + (1 - g) * b
```

```python
import numpy as np
import jax
import jax.numpy as jnp
import jax.experimental.pallas as pl
import jax.experimental.pallas.tpu as pltpu

S = 2048
D = 640
KS = 4
C = 256
N2 = 2 * C
H = C // 2
NB = S // C
DT = 128
SH = S // 2


def _dft_mats():
    kperm = np.concatenate([np.arange(0, H, 2), np.arange(1, H, 2)])
    phi = 2.0 * np.pi * (kperm + 0.5) / N2
    se = np.arange(0, C, 2)
    so = np.arange(1, C, 2)
    fe = np.concatenate([np.cos(phi[:, None] * se[None]), -np.sin(phi[:, None] * se[None])], 0)
    fo = np.concatenate([np.cos(phi[:, None] * so[None]), -np.sin(phi[:, None] * so[None])], 0)
    ie = (2.0 / N2) * np.concatenate(
        [np.cos(phi[None] * se[:, None]), -np.sin(phi[None] * se[:, None])], 1)
    io = (2.0 / N2) * np.concatenate(
        [np.cos(phi[None] * so[:, None]), -np.sin(phi[None] * so[:, None])], 1)
    cast = lambda a: jnp.asarray(a.astype(np.float32)).astype(jnp.bfloat16)
    return cast(fe), cast(fo), cast(ie), cast(io)


def _split(x_bf16):
    u = pltpu.bitcast(x_bf16, jnp.uint32)
    ev = pltpu.bitcast(u << 16, jnp.float32)
    od = pltpu.bitcast(u & jnp.uint32(0xFFFF0000), jnp.float32)
    return ev, od


def _merge(ev_f32, od_f32):
    eb = pltpu.bitcast(ev_f32.astype(jnp.bfloat16).astype(jnp.float32), jnp.uint32)
    ob = pltpu.bitcast(od_f32.astype(jnp.bfloat16).astype(jnp.float32), jnp.uint32)
    u = (eb >> 16) | (ob & jnp.uint32(0xFFFF0000))
    return pltpu.bitcast(u, jnp.bfloat16)


def _rb(x):
    return x.astype(jnp.bfloat16).astype(jnp.float32)


def _shift_down(x, n):
    r = pltpu.roll(x, n, axis=0)
    rows = jax.lax.broadcasted_iota(jnp.int32, x.shape, 0)
    return jnp.where(rows >= n, r, 0.0)


def _blocks_to_lanes(x):
    return jnp.concatenate([x[b * H:(b + 1) * H, :] for b in range(NB)], axis=1)


def _lanes_to_blocks(x):
    return jnp.concatenate([x[:, b * DT:(b + 1) * DT] for b in range(NB)], axis=0)


def _kernel(q_ref, gw_ref, ak_ref, av_ref, bk_ref, bv_ref, ash_ref, bsh_ref,
            ah_ref, bh_ref, ad_ref, bd_ref, fe_ref, fo_ref, ie_ref, io_ref,
            o_ref,
            ge_scr, go_scr, xe_scr, xo_scr, he_scr, ho_scr, ye_scr, yo_scr):
    step = pl.program_id(0)

    @pl.when(step == 0)
    def _():
        qe, qo = _split(q_ref[...])
        gw = gw_ref[...]
        le = jnp.dot(qe.astype(jnp.bfloat16), gw, preferred_element_type=jnp.float32)
        lo = jnp.dot(qo.astype(jnp.bfloat16), gw, preferred_element_type=jnp.float32)
        ge_scr[...] = jax.nn.sigmoid(le)
        go_scr[...] = jax.nn.sigmoid(lo)

    fe = fe_ref[...]
    fo = fo_ref[...]
    ie = ie_ref[...]
    io = io_ref[...]

    col = pl.multiple_of(step * DT, DT)
    qe, qo = _split(q_ref[:, pl.ds(col, DT)])

    def branch(k_ref, v_ref, sh_ref, h_ref, d_ref):
        ke, ko = _split(k_ref[...])
        ve, vo = _split(v_ref[...])
        w = sh_ref[...].astype(jnp.float32)
        w0, w1, w2, w3 = w[0:1], w[1:2], w[2:3], w[3:4]
        ke1 = _shift_down(ke, 1)
        ko1 = _shift_down(ko, 1)
        ko2 = _shift_down(ko, 2)
        kse = ke * w0 + ko1 * w1 + ke1 * w2 + ko2 * w3
        kso = ko * w0 + ke * w1 + ko1 * w2 + ke1 * w3
        kve = _rb(_rb(kse) * ve)
        kvo = _rb(_rb(kso) * vo)

        xe_scr[...] = jnp.dot(fe, _blocks_to_lanes(kve.astype(jnp.bfloat16)),
                              preferred_element_type=jnp.float32)
        xo_scr[...] = jnp.dot(fo, _blocks_to_lanes(kvo.astype(jnp.bfloat16)),
                              preferred_element_type=jnp.float32)
        ht = h_ref[...].T
        hte, hto = _split(ht)
        he_scr[...] = jnp.dot(fe, _blocks_to_lanes(hte.astype(jnp.bfloat16)),
                              preferred_element_type=jnp.float32)
        ho_scr[...] = jnp.dot(fo, _blocks_to_lanes(hto.astype(jnp.bfloat16)),
                              preferred_element_type=jnp.float32)

        def make_body(sign):
            def body(i, carry):
                r = pl.multiple_of(i * 8, 8)
                rr = pl.ds(r, 8)
                ri = pl.ds(r + H, 8)

                def ld(ref, rows, b):
                    return ref[rows, b * DT:(b + 1) * DT]

                res = []
                for s_uv in (1.0, -1.0):
                    def comb(a, b_):
                        return a + b_ if s_uv > 0 else a - b_
                    xr = [comb(ld(xe_scr, rr, b), ld(xo_scr, rr, b)) for b in range(NB)]
                    xi = [comb(ld(xe_scr, ri, b), ld(xo_scr, ri, b)) for b in range(NB)]
                    hr = [comb(ld(he_scr, rr, b), ld(ho_scr, rr, b)) for b in range(NB)]
                    hi = [comb(ld(he_scr, ri, b), ld(ho_scr, ri, b)) for b in range(NB)]
                    gr = [hr[0]]
                    gi = [hi[0]]
                    for j in range(1, NB):
                        if sign > 0:
                            gr.append(hr[j] - hi[j - 1])
                            gi.append(hi[j] + hr[j - 1])
                        else:
                            gr.append(hr[j] + hi[j - 1])
                            gi.append(hi[j] - hr[j - 1])
                    yr = []
                    yi = []
                    for b in range(NB):
                        accr = None
                        acci = None
                        for j in range(b + 1):
                            tr = xr[b - j] * gr[j] - xi[b - j] * gi[j]
                            ti = xr[b - j] * gi[j] + xi[b - j] * gr[j]
                            accr = tr if accr is None else accr + tr
                            acci = ti if acci is None else acci + ti
                        yr.append(accr)
                        yi.append(acci)
                    res.append((yr, yi))
                (ur, ui), (vr, vi) = res
                for b in range(NB):
                    ye_scr[rr, b * DT:(b + 1) * DT] = ur[b] + vr[b]
                    ye_scr[ri, b * DT:(b + 1) * DT] = ui[b] + vi[b]
                    yo_scr[rr, b * DT:(b + 1) * DT] = ur[b] - vr[b]
                    yo_scr[ri, b * DT:(b + 1) * DT] = ui[b] - vi[b]
                return carry
            return body

        nchunk = H // 8
        jax.lax.fori_loop(0, nchunk // 2, make_body(1), 0)
        jax.lax.fori_loop(nchunk // 2, nchunk, make_body(-1), 0)

        ye = _lanes_to_blocks(jnp.dot(ie, ye_scr[...].astype(jnp.bfloat16),
                                      preferred_element_type=jnp.float32))
        yo = _lanes_to_blocks(jnp.dot(io, yo_scr[...].astype(jnp.bfloat16),
                                      preferred_element_type=jnp.float32))
        dd = d_ref[...].astype(jnp.float32)
        ye = _rb(_rb(ye) + _rb(kve * dd))
        yo = _rb(_rb(yo) + _rb(kvo * dd))
        return _rb(qe * ye), _rb(qo * yo)

    ae, ao = branch(ak_ref, av_ref, ash_ref, ah_ref, ad_ref)
    be, bo = branch(bk_ref, bv_ref, bsh_ref, bh_ref, bd_ref)
    ge = ge_scr[...]
    go = go_scr[...]
    oe = ge * ae + (1.0 - ge) * be
    oo = go * ao + (1.0 - go) * bo
    o_ref[...] = _merge(oe, oo)


@jax.jit
def pallas_gated_mix__ssm_conv_h3__ssm_conv_h3__prompt_kernel(
    A_q: jax.Array,
    A_k: jax.Array,
    A_v: jax.Array,
    A_shift_k: jax.Array,
    A_ssm_k: jax.Array,
    A_ssm_D: jax.Array,
    B_q: jax.Array,
    B_k: jax.Array,
    B_v: jax.Array,
    B_shift_k: jax.Array,
    B_ssm_k: jax.Array,
    B_ssm_D: jax.Array,
    gate_w: jax.Array,
):
    q = A_q.reshape(S, D)
    ak = A_k.reshape(S, D)
    av = A_v.reshape(S, D)
    bk = B_k.reshape(S, D)
    bv = B_v.reshape(S, D)
    ash = A_shift_k.T
    bsh = B_shift_k.T
    ad = A_ssm_D.reshape(1, D)
    bd = B_ssm_D.reshape(1, D)
    gw = jnp.broadcast_to(gate_w.reshape(D, 1), (D, DT))
    fe, fo, ie, io = _dft_mats()

    tile = lambda: pl.BlockSpec((S, DT), lambda i: (0, i))
    full = lambda shp: pl.BlockSpec(shp, lambda i: (0,) * len(shp))
    in_specs = [
        full((S, D)),
        full((D, DT)),
        tile(), tile(), tile(), tile(),
        pl.BlockSpec((KS, DT), lambda i: (0, i)),
        pl.BlockSpec((KS, DT), lambda i: (0, i)),
        pl.BlockSpec((DT, S), lambda i: (i, 0)),
        pl.BlockSpec((DT, S), lambda i: (i, 0)),
        pl.BlockSpec((1, DT), lambda i: (0, i)),
        pl.BlockSpec((1, DT), lambda i: (0, i)),
        full((2 * H, H)), full((2 * H, H)), full((H, 2 * H)), full((H, 2 * H)),
    ]
    scratch = [
        pltpu.VMEM((SH, DT), jnp.float32),
        pltpu.VMEM((SH, DT), jnp.float32),
        pltpu.VMEM((2 * H, NB * DT), jnp.float32),
        pltpu.VMEM((2 * H, NB * DT), jnp.float32),
        pltpu.VMEM((2 * H, NB * DT), jnp.float32),
        pltpu.VMEM((2 * H, NB * DT), jnp.float32),
        pltpu.VMEM((2 * H, NB * DT), jnp.float32),
        pltpu.VMEM((2 * H, NB * DT), jnp.float32),
    ]
    out = pl.pallas_call(
        _kernel,
        grid=(D // DT,),
        in_specs=in_specs,
        out_specs=pl.BlockSpec((S, DT), lambda i: (0, i)),
        out_shape=jax.ShapeDtypeStruct((S, D), jnp.bfloat16),
        scratch_shapes=scratch,
        compiler_params=pltpu.CompilerParams(
            dimension_semantics=("arbitrary",),
            vmem_limit_bytes=100 * 1024 * 1024,
        ),
    )(q, gw, ak, av, bk, bv, ash, bsh, A_ssm_k, B_ssm_k, ad, bd, fe, fo, ie, io)
    return out.reshape(1, S, D)
```

```python
import numpy as np
import jax
import jax.numpy as jnp
import jax.experimental.pallas as pl
import jax.experimental.pallas.tpu as pltpu

S = 2048
D = 640
KS = 4
C = 256
N2 = 2 * C
H = C // 2
NB = S // C
DT = 128
NT = D // DT
f32 = jnp.float32
bf16 = jnp.bfloat16


def _dft_mats():
    kperm = np.concatenate([np.arange(0, H, 2), np.arange(1, H, 2)])
    phi = 2.0 * np.pi * (kperm + 0.5) / N2
    se = np.arange(0, C, 2)
    so = np.arange(1, C, 2)
    fe = np.concatenate([np.cos(phi[:, None] * se[None]), -np.sin(phi[:, None] * se[None])], 0)
    fo = np.concatenate([np.cos(phi[:, None] * so[None]), -np.sin(phi[:, None] * so[None])], 0)
    ie = (2.0 / N2) * np.concatenate(
        [np.cos(phi[None] * se[:, None]), -np.sin(phi[None] * se[:, None])], 1)
    io = (2.0 / N2) * np.concatenate(
        [np.cos(phi[None] * so[:, None]), -np.sin(phi[None] * so[:, None])], 1)
    def cast(a):
        u = np.ascontiguousarray(a.astype(np.float32)).view(np.uint32).astype(np.uint64)
        r = ((u + 0x7FFF + ((u >> 16) & 1)) >> 16).astype(np.uint32)
        return jnp.asarray(r[0::2] | (r[1::2] << 16))
    return cast(fe), cast(fo), cast(ie), cast(io)


def _lo(u):
    return pltpu.bitcast(u << 16, f32)


def _hi(u):
    return pltpu.bitcast(u & jnp.uint32(0xFFFF0000), f32)


def _split(x_bf16):
    u = pltpu.bitcast(x_bf16, jnp.uint32)
    return _lo(u), _hi(u)


def _merge(ev_f32, od_f32):
    eb = pltpu.bitcast(ev_f32.astype(bf16).astype(f32), jnp.uint32)
    ob = pltpu.bitcast(od_f32.astype(bf16).astype(f32), jnp.uint32)
    u = (eb >> 16) | (ob & jnp.uint32(0xFFFF0000))
    return pltpu.bitcast(u, bf16)


def _pk(x_bf16):
    return pltpu.bitcast(x_bf16, jnp.uint32)


def _upk(u):
    return pltpu.bitcast(u, bf16)


def _dot(a, b):
    return jnp.dot(a, b, preferred_element_type=f32)


def _kernel(q_hbm, gw_ref, ak_ref, av_ref, bk_ref, bv_ref, ash_ref, bsh_ref,
            ah_ref, bh_ref, ad_ref, bd_ref, fe_ref, fo_ref, ie_ref, io_ref,
            o_ref,
            q_vmem, q_sem, g_scr, xa, ha, ya, kva, xb, hb, yb, kvb, a_scr,
            hs_scr, yi_scr, d_scr):
    t = pl.program_id(0)

    def stage_p(b, first, k_ref, v_ref, sh_ref, h_ref, kv_scr, slot):
        r0 = pl.multiple_of(b * C, C)
        ku = pltpu.bitcast(k_ref[pl.ds(r0, C), :], jnp.uint32)
        if first:
            halo = jnp.zeros((8, DT), jnp.uint32)
        else:
            halo = pltpu.bitcast(k_ref[pl.ds(pl.multiple_of(r0 - 16, 16), 16), :], jnp.uint32)
        ext = jnp.concatenate([halo, ku], axis=0)
        kee = _lo(ext)
        koe = _hi(ext)
        ke = kee[8:]
        ko = koe[8:]
        ke1 = kee[7:7 + H]
        ko1 = koe[7:7 + H]
        ko2 = koe[6:6 + H]
        ve, vo = _split(v_ref[pl.ds(r0, C), :])
        w = sh_ref[...].astype(f32)
        w0, w1, w2, w3 = w[0:1], w[1:2], w[2:3], w[3:4]
        kse = ke * w0 + ko1 * w1 + ke1 * w2 + ko2 * w3
        kso = ko * w0 + ke * w1 + ko1 * w2 + ke1 * w3
        kv_scr[slot, b, 0] = _pk((kse * ve).astype(bf16))
        kv_scr[slot, b, 1] = _pk((kso * vo).astype(bf16))
        ht = h_ref[:, pl.ds(r0, C)].T
        hte, hto = _split(ht)
        hs_scr[b, 0] = _pk(hte.astype(bf16))
        hs_scr[b, 1] = _pk(hto.astype(bf16))

    def stage_f(b, kv_scr, slot, x_scr, h_scr):
        fe = _upk(fe_ref[...])
        fo = _upk(fo_ref[...])
        e = _dot(fe, _upk(kv_scr[slot, b, 0]))
        o = _dot(fo, _upk(kv_scr[slot, b, 1]))
        x_scr[b, 0] = e + o
        x_scr[b, 1] = e - o
        e = _dot(fe, _upk(hs_scr[b, 0]))
        o = _dot(fo, _upk(hs_scr[b, 1]))
        h_scr[b, 0] = e + o
        h_scr[b, 1] = e - o

    def stage_w(chunk, sign, x_scr, h_scr, y_scr):
        r = pl.multiple_of(chunk * 8, 8)
        rr = pl.ds(r, 8)
        ri = pl.ds(r + H, 8)
        for uv in (0, 1):
            xr = [x_scr[j, uv, rr, :] for j in range(NB)]
            xi = [x_scr[j, uv, ri, :] for j in range(NB)]
            hr = [h_scr[j, uv, rr, :] for j in range(NB)]
            hi = [h_scr[j, uv, ri, :] for j in range(NB)]
            gr = [hr[0]]
            gi = [hi[0]]
            for j in range(1, NB):
                if sign > 0:
                    gr.append(hr[j] - hi[j - 1])
                    gi.append(hi[j] + hr[j - 1])
                else:
                    gr.append(hr[j] + hi[j - 1])
                    gi.append(hi[j] - hr[j - 1])
            for bb in range(NB):
                accr = None
                acci = None
                for j in range(bb + 1):
                    tr = xr[bb - j] * gr[j] - xi[bb - j] * gi[j]
                    ti = xr[bb - j] * gi[j] + xi[bb - j] * gr[j]
                    accr = tr if accr is None else accr + tr
                    acci = ti if acci is None else acci + ti
                y_scr[bb, uv, rr, :] = accr
                y_scr[bb, uv, ri, :] = acci

    def stage_i(b, y_scr):
        u = y_scr[b, 0]
        v = y_scr[b, 1]
        yi_scr[b, 0] = _dot(_upk(ie_ref[...]), (u + v).astype(bf16))
        yi_scr[b, 1] = _dot(_upk(io_ref[...]), (u - v).astype(bf16))

    def stage_q(b, tile, kv_scr, slot, d_ref, is_b):
        r0 = pl.multiple_of(b * C, C)
        col = pl.multiple_of(tile * DT, DT)
        dd = d_scr[d_ref:d_ref + 1, pl.ds(col, DT)]
        qe, qo = _split(q_vmem[pl.ds(r0, C), pl.ds(col, DT)])
        re_ = qe * (yi_scr[b, 0] + _upk(kv_scr[slot, b, 0]).astype(f32) * dd)
        ro_ = qo * (yi_scr[b, 1] + _upk(kv_scr[slot, b, 1]).astype(f32) * dd)
        if not is_b:
            a_scr[b, 0] = re_
            a_scr[b, 1] = ro_
        else:
            oe = re_ + g_scr[b, 0] * (a_scr[b, 0] - re_)
            oo = ro_ + g_scr[b, 1] * (a_scr[b, 1] - ro_)
            o_ref[pl.ds(r0, C), :] = _merge(oe, oo)

    par = t % 2

    p_a = lambda b, first: stage_p(b, first, ak_ref, av_ref, ash_ref, ah_ref, kva, par)
    p_b = lambda b, first: stage_p(b, first, bk_ref, bv_ref, bsh_ref, bh_ref, kvb, par)

    q_copy = pltpu.make_async_copy(q_hbm, q_vmem, q_sem)

    def stage_g(b):
        r0 = pl.multiple_of(b * C, C)
        gwb = jnp.broadcast_to(gw_ref[...].reshape(1, D), (DT, D))
        qe, qo = _split(q_vmem[pl.ds(r0, C), :])
        dn = (((1,), (1,)), ((), ()))
        le = jax.lax.dot_general(qe.astype(bf16), gwb, dn, preferred_element_type=f32)
        lo = jax.lax.dot_general(qo.astype(bf16), gwb, dn, preferred_element_type=f32)
        g_scr[b, 0] = jax.nn.sigmoid(le)
        g_scr[b, 1] = jax.nn.sigmoid(lo)

    @pl.when(t == 0)
    def _():
        q_copy.start()
        d_scr[0:1, :] = ad_ref[...].reshape(1, D).astype(f32)
        d_scr[1:2, :] = bd_ref[...].reshape(1, D).astype(f32)
        p_a(0, True)

        def loop_0(b, c):
            stage_f(b, kva, par, xa, ha)
            p_a(jnp.minimum(b + 1, NB - 1), False)
            return c
        jax.lax.fori_loop(0, NB, loop_0, 0)

    @pl.when(t == 1)
    def _():
        q_copy.wait()
        p_b(0, True)

        def loop_a1(b, c):
            bn = jnp.minimum(b + 1, NB - 1)
            stage_f(b, kvb, par, xb, hb)
            stage_g(b)
            p_b(bn, False)
            stage_w(b, 1, xa, ha, ya)
            stage_w(b + NB, -1, xa, ha, ya)
            return c

        jax.lax.fori_loop(0, NB, loop_a1, 0)

    @pl.when(jnp.logical_and(t >= 2, t <= NT))
    def _():
        p_b(0, True)
        stage_i(0, yb)

        def loop_a(b, c):
            bn = jnp.minimum(b + 1, NB - 1)
            stage_f(b, kvb, par, xb, hb)
            stage_i(bn, yb)
            stage_q(b, t - 2, kvb, 1 - par, 1, True)
            p_b(bn, False)
            stage_w(b, 1, xa, ha, ya)
            stage_w(b + NB, -1, xa, ha, ya)
            return c

        jax.lax.fori_loop(0, NB, loop_a, 0)

    @pl.when(jnp.logical_and(t >= 1, t <= NT))
    def _():
        p_a(0, True)
        stage_i(0, ya)

        def loop_b(b, c):
            bn = jnp.minimum(b + 1, NB - 1)
            stage_f(b, kva, par, xa, ha)
            stage_i(bn, ya)
            stage_q(b, t - 1, kva, 1 - par, 0, False)
            p_a(bn, False)
            stage_w(b, 1, xb, hb, yb)
            stage_w(b + NB, -1, xb, hb, yb)
            return c

        jax.lax.fori_loop(0, NB, loop_b, 0)

    @pl.when(t == NT + 1)
    def _():
        def loop_e(b, c):
            stage_i(b, yb)
            stage_q(b, NT - 1, kvb, 1 - par, 1, True)
            return c
        jax.lax.fori_loop(0, NB, loop_e, 0)


@jax.jit
def pallas_gated_mix__ssm_conv_h3__ssm_conv_h3__prompt_kernel(
    A_q: jax.Array,
    A_k: jax.Array,
    A_v: jax.Array,
    A_shift_k: jax.Array,
    A_ssm_k: jax.Array,
    A_ssm_D: jax.Array,
    B_q: jax.Array,
    B_k: jax.Array,
    B_v: jax.Array,
    B_shift_k: jax.Array,
    B_ssm_k: jax.Array,
    B_ssm_D: jax.Array,
    gate_w: jax.Array,
):
    q = A_q.reshape(S, D)
    ak = A_k.reshape(S, D)
    av = A_v.reshape(S, D)
    bk = B_k.reshape(S, D)
    bv = B_v.reshape(S, D)
    ash = A_shift_k.T
    bsh = B_shift_k.T
    ad = A_ssm_D
    bd = B_ssm_D
    gw = gate_w
    fe, fo, ie, io = _dft_mats()

    ia = lambda t: jnp.minimum(t, NT - 1)
    ib = lambda t: jnp.clip(t - 1, 0, NT - 1)
    iad = lambda t: jnp.clip(t - 1, 0, NT - 1)
    ibd = lambda t: jnp.clip(t - 2, 0, NT - 1)
    full = lambda shp: pl.BlockSpec(shp, lambda t: (0,) * len(shp))
    in_specs = [
        pl.BlockSpec(memory_space=pl.ANY),
        full((D,)),
        pl.BlockSpec((S, DT), lambda t: (0, ia(t))),
        pl.BlockSpec((S, DT), lambda t: (0, ia(t))),
        pl.BlockSpec((S, DT), lambda t: (0, ib(t))),
        pl.BlockSpec((S, DT), lambda t: (0, ib(t))),
        pl.BlockSpec((KS, DT), lambda t: (0, ia(t))),
        pl.BlockSpec((KS, DT), lambda t: (0, ib(t))),
        pl.BlockSpec((DT, S), lambda t: (ia(t), 0)),
        pl.BlockSpec((DT, S), lambda t: (ib(t), 0)),
        full((D,)),
        full((D,)),
        full((H, H)), full((H, H)), full((H // 2, 2 * H)), full((H // 2, 2 * H)),
    ]
    spec = lambda: pltpu.VMEM((NB, 2, 2 * H, DT), f32)
    scratch = [
        pltpu.VMEM((S, D), bf16),
        pltpu.SemaphoreType.DMA(()),
        pltpu.VMEM((NB, 2, H, DT), f32),
        spec(), spec(), spec(),
        pltpu.VMEM((2, NB, 2, H // 2, DT), jnp.uint32),
        spec(), spec(), spec(),
        pltpu.VMEM((2, NB, 2, H // 2, DT), jnp.uint32),
        pltpu.VMEM((NB, 2, H, DT), f32),
        pltpu.VMEM((NB, 2, H // 2, DT), jnp.uint32),
        pltpu.VMEM((NB, 2, H, DT), f32),
        pltpu.VMEM((8, D), f32),
    ]
    out = pl.pallas_call(
        _kernel,
        grid=(NT + 2,),
        in_specs=in_specs,
        out_specs=pl.BlockSpec((S, DT), lambda t: (0, ibd(t))),
        out_shape=jax.ShapeDtypeStruct((S, D), bf16),
        scratch_shapes=scratch,
        compiler_params=pltpu.CompilerParams(
            dimension_semantics=("arbitrary",),
            vmem_limit_bytes=100 * 1024 * 1024,
        ),
    )(q, gw, ak, av, bk, bv, ash, bsh, A_ssm_k, B_ssm_k, ad, bd, fe, fo, ie, io)
    return out.reshape(1, S, D)
```
